```python
import os as _os
_os.environ.setdefault("JAX_PLATFORMS", "cpu")
import jax
import jax.numpy as jnp

def _softmax(x, axis=-1):
    return jax.nn.softmax(x, axis=axis)
def _gelu(x):
    return jax.nn.gelu(x, approximate=True)
def _silu(x):
    return jax.nn.silu(x)
def _sigmoid(x):
    return jax.nn.sigmoid(x)
def _layernorm(x, axis=-1, eps=1e-5):
    m = jnp.mean(x, axis=axis, keepdims=True)
    v = jnp.var(x, axis=axis, keepdims=True)
    return (x - m) / jnp.sqrt(v + eps)
def _scatter_add(tgt, idx, src, axis=0):
    return tgt.at[idx].add(src)
def _segment_sum(src, seg, n):
    return jax.ops.segment_sum(src, seg, n)
class _Rng:
    def __init__(self, key):
        self._k = key
    def _next(self):
        self._k, sub = jax.random.split(self._k)
        return sub
    def normal(self, shape):
        return jax.random.normal(self._next(), shape, dtype=jnp.bfloat16)
    def randint(self, lo, hi, shape):
        return jax.random.randint(self._next(), shape, lo, hi, dtype=jnp.int32)
    def uniform(self, shape, lo=0.0, hi=1.0):
        return jax.random.uniform(self._next(), shape, jnp.bfloat16, lo, hi)
    def permutation(self, n):
        return jax.random.permutation(self._next(), n)


kernel_name = 'concat_heads__sliding_block_cached__sliding_block_cached__decode'

def setup_inputs():
    _rng = _Rng(jax.random.key(int.from_bytes(__import__("os").urandom(4), "little")))
    _w = (lambda a: (lambda t: t.astype(jnp.bfloat16) if jnp.issubdtype(t.dtype, jnp.floating) else t)(jnp.asarray(a)))
    def _A_setup():
        B, Sq, D = 2, 1, 640
        Hq, Hkv, Sk, Dh = 32, 32, 4096, 128
        assert Hq % Hkv == 0, (Hq, Hkv)
        return {
            "x": _w((lambda *s: _rng.normal(s) * 0.8)(B, Sq, D)),
            "k_cache": _w((lambda *s: _rng.normal(s) * 0.8)(B, Hkv, Sk, Dh)),
            "v_cache": _w((lambda *s: _rng.normal(s) * 0.05)(B, Hkv, Sk, Dh)),
            "wq": _w((lambda *s: _rng.normal(s) * 0.8)(D, Hq * Dh) * (D ** -0.5)),
            "wo": _w((lambda *s: _rng.normal(s) * 0.05)(Hq * Dh, D) * ((Hq * Dh) ** -0.5)),
        }
    _A_in = _A_setup()

    def _B_setup():
        B, Sq, D = 2, 1, 640
        Hq, Hkv, Sk, Dh = 32, 32, 4096, 128
        assert Hq % Hkv == 0, (Hq, Hkv)
        return {
            "x": _w((lambda *s: _rng.normal(s) * 0.8)(B, Sq, D)),
            "k_cache": _w((lambda *s: _rng.normal(s) * 0.8)(B, Hkv, Sk, Dh)),
            "v_cache": _w((lambda *s: _rng.normal(s) * 0.05)(B, Hkv, Sk, Dh)),
            "wq": _w((lambda *s: _rng.normal(s) * 0.8)(D, Hq * Dh) * (D ** -0.5)),
            "wo": _w((lambda *s: _rng.normal(s) * 0.05)(Hq * Dh, D) * ((Hq * Dh) ** -0.5)),
        }
    _B_in = _B_setup()

    return {
        "A_x": _A_in["x"],
        "A_k_cache": _A_in["k_cache"],
        "A_v_cache": _A_in["v_cache"],
        "A_wq": _A_in["wq"],
        "A_wo": _A_in["wo"],
        "B_x": _B_in["x"],
        "B_k_cache": _B_in["k_cache"],
        "B_v_cache": _B_in["v_cache"],
        "B_wq": _B_in["wq"],
        "B_wo": _B_in["wo"],
    }

def reference(A_x, A_k_cache, A_v_cache, A_wq, A_wo, B_x, B_k_cache, B_v_cache, B_wq, B_wo):
    def _A_ref(x, k_cache, v_cache, wq, wo):
        B, Sq, D = x.shape
        Hq, Dh = 32, 128
        Hkv, Sk = k_cache.shape[1], k_cache.shape[2]
        W = min(4096, max(256, Sk // 4))
        rep = Hq // Hkv
        q = (lambda x, *d: x.transpose(*d))((x @ wq).reshape(B, Sq, Hq, Dh), 0, 2, 1, 3)
        k = jnp.repeat(k_cache[:, :, Sk - W:, :], rep, axis=1)
        v = jnp.repeat(v_cache[:, :, Sk - W:, :], rep, axis=1)
        scores = jnp.einsum("bhqd,bhkd->bhqk", q, k) * (Dh ** -0.5)
        p = _softmax(scores, axis=-1)
        o = jnp.einsum("bhqk,bhkd->bhqd", p, v)
        return (lambda x, *d: x.transpose(*d))(o, 0, 2, 1, 3).reshape(B, Sq, Hq * Dh) @ wo

    def _B_ref(x, k_cache, v_cache, wq, wo):
        B, Sq, D = x.shape
        Hq, Dh = 32, 128
        Hkv, Sk = k_cache.shape[1], k_cache.shape[2]
        W = min(4096, max(256, Sk // 4))
        rep = Hq // Hkv
        q = (lambda x, *d: x.transpose(*d))((x @ wq).reshape(B, Sq, Hq, Dh), 0, 2, 1, 3)
        k = jnp.repeat(k_cache[:, :, Sk - W:, :], rep, axis=1)
        v = jnp.repeat(v_cache[:, :, Sk - W:, :], rep, axis=1)
        scores = jnp.einsum("bhqd,bhkd->bhqk", q, k) * (Dh ** -0.5)
        p = _softmax(scores, axis=-1)
        o = jnp.einsum("bhqk,bhkd->bhqd", p, v)
        return (lambda x, *d: x.transpose(*d))(o, 0, 2, 1, 3).reshape(B, Sq, Hq * Dh) @ wo

    a = _A_ref(A_x, A_k_cache, A_v_cache, A_wq, A_wo)
    b = _B_ref(B_x, B_k_cache, B_v_cache, B_wq, B_wo)
    return jnp.concatenate([a, b], axis=-1)
```

```python
import functools

import jax
import jax.numpy as jnp
import jax.experimental.pallas as pl
import jax.experimental.pallas.tpu as pltpu

_HG = 1


def _branch(x_ref, k_ref, v_ref, wq_ref, wo_ref, *, hg, dh, scale):
    nb = x_ref.shape[0]
    x = jnp.concatenate([x_ref[b] for b in range(nb)], axis=0)
    q = jnp.dot(x, wq_ref[...], preferred_element_type=jnp.float32)
    q = q.astype(jnp.bfloat16)
    rows = []
    for b in range(nb):
        cols = []
        for h in range(hg):
            qb = q[b:b + 1, h * dh:(h + 1) * dh]
            s = jax.lax.dot_general(
                qb, k_ref[b, h], (((1,), (1,)), ((), ())),
                preferred_element_type=jnp.float32) * scale
            m = jnp.max(s, axis=-1, keepdims=True)
            p = jnp.exp(s - m)
            l = jnp.sum(p, axis=-1, keepdims=True)
            o = jnp.dot(p.astype(jnp.bfloat16), v_ref[b, h],
                        preferred_element_type=jnp.float32)
            cols.append(o / l)
        rows.append(jnp.concatenate(cols, axis=1) if hg > 1 else cols[0])
    o_all = jnp.concatenate(rows, axis=0).astype(jnp.bfloat16)
    return jnp.dot(o_all, wo_ref[...], preferred_element_type=jnp.float32)


def _kernel(ax, ak, av, awq, awo, bx, bk, bv, bwq, bwo, o_ref, acc_a, acc_b,
            *, hg, dh, scale):
    g = pl.program_id(0)

    @pl.when(g == 0)
    def _():
        acc_a[...] = jnp.zeros_like(acc_a)
        acc_b[...] = jnp.zeros_like(acc_b)

    acc_a[...] += _branch(ax, ak, av, awq, awo, hg=hg, dh=dh, scale=scale)
    acc_b[...] += _branch(bx, bk, bv, bwq, bwo, hg=hg, dh=dh, scale=scale)

    @pl.when(g == pl.num_programs(0) - 1)
    def _():
        d = acc_a.shape[1]
        for b in range(acc_a.shape[0]):
            o_ref[b, :, 0:d] = acc_a[b:b + 1, :].astype(o_ref.dtype)
            o_ref[b, :, d:2 * d] = acc_b[b:b + 1, :].astype(o_ref.dtype)


@jax.jit
def pallas_concat_heads__sliding_block_cached__sliding_block_cached__decode_kernel(
    A_x: jax.Array,
    A_k_cache: jax.Array,
    A_v_cache: jax.Array,
    A_wq: jax.Array,
    A_wo: jax.Array,
    B_x: jax.Array,
    B_k_cache: jax.Array,
    B_v_cache: jax.Array,
    B_wq: jax.Array,
    B_wo: jax.Array,
):
    B, Sq, D = A_x.shape
    _, H, Sk, Dh = A_k_cache.shape
    W = min(4096, max(256, Sk // 4))
    assert Sq == 1 and Sk % W == 0
    wblk = (Sk - W) // W
    hg = _HG
    scale = Dh ** -0.5

    x_spec = pl.BlockSpec((B, Sq, D), lambda g: (0, 0, 0))
    kv_spec = pl.BlockSpec((B, hg, W, Dh), lambda g: (0, g, wblk, 0))
    wq_spec = pl.BlockSpec((D, hg * Dh), lambda g: (0, g))
    wo_spec = pl.BlockSpec((hg * Dh, D), lambda g: (g, 0))
    specs = [x_spec, kv_spec, kv_spec, wq_spec, wo_spec]

    return pl.pallas_call(
        functools.partial(_kernel, hg=hg, dh=Dh, scale=scale),
        grid=(H // hg,),
        in_specs=specs + specs,
        out_specs=pl.BlockSpec((B, Sq, 2 * D), lambda g: (0, 0, 0)),
        out_shape=jax.ShapeDtypeStruct((B, Sq, 2 * D), A_x.dtype),
        scratch_shapes=[pltpu.VMEM((B, D), jnp.float32), pltpu.VMEM((B, D), jnp.float32)],
        compiler_params=pltpu.CompilerParams(
            dimension_semantics=("arbitrary",),
            vmem_limit_bytes=64 * 1024 * 1024,
        ),
    )(A_x, A_k_cache, A_v_cache, A_wq, A_wo, B_x, B_k_cache, B_v_cache, B_wq, B_wo)
```

```python
import functools

import jax
import jax.numpy as jnp
import jax.experimental.pallas as pl
import jax.experimental.pallas.tpu as pltpu

_KV_SPLIT = 8
_WO_SPLIT = 4
_LOOKAHEAD = 72
_TAIL_FIFO = 72
_NSLOT = 2
_WQ_ROWS = 8
_WQ_COLS = 2048
_WQ_KB = 128
_WQ_SEMS = 128


def _kernel(ax, ak, av, awq, awo, bx, bk, bv, bwq, bwo, o_ref,
            x_buf, wq_buf, k_buf, v_buf, wo_buf, q_acc, acc, x_sem, wq_sems, sems,
            *, nb, nh, dh, d, w, s0, scale):
    xs, ks, vs, wqs, wos = (ax, bx), (ak, bk), (av, bv), (awq, bwq), (awo, bwo)
    kvr = w // _KV_SPLIT
    wor = dh // _WO_SPLIT
    pairs = [(br, b) for br in range(2) for b in range(nb)]
    L = _LOOKAHEAD
    assert L < _WQ_SEMS

    wq_subs = [(br, kb + rr, cc, rr == _WQ_KB - _WQ_ROWS)
               for br in range(2) for kb in range(0, d, _WQ_KB)
               for cc in range(0, nh * dh, _WQ_COLS) for rr in range(0, _WQ_KB, _WQ_ROWS)]
    nwq = len(wq_subs)
    assert nwq % 2 == 0

    subs = []
    for br, b in pairs:
        subs += [("k", br, b, p, p == _KV_SPLIT - 1) for p in range(_KV_SPLIT)]
    for br, b in pairs:
        subs += [("v", br, b, p, p == _KV_SPLIT - 1) for p in range(_KV_SPLIT)]
    for br in range(2):
        subs += [("wo", br, 0, p, br == 1 and p == _WO_SPLIT - 1) for p in range(_WO_SPLIT)]
    nsub = len(subs)
    assert L <= (_NSLOT - 1) * nsub and nsub % 2 == 0
    total = nh * nsub

    def wq_copy(i):
        br, r0, c0, _ = wq_subs[i]
        return pltpu.make_async_copy(
            wqs[br].at[pl.ds(r0, _WQ_ROWS), pl.ds(c0, _WQ_COLS)],
            wq_buf.at[br, pl.ds(r0, _WQ_ROWS), pl.ds(c0, _WQ_COLS)],
            wq_sems.at[i % _WQ_SEMS])

    def copy(h, j):
        kind, br, b, p, _ = subs[j]
        slot = h % _NSLOT
        if kind == "wo":
            src = wos[br].at[pl.ds(pl.multiple_of(h * dh + p * wor, wor), wor), :]
            dst = wo_buf.at[slot, br, pl.ds(p * wor, wor), :]
        elif kind == "k":
            src = ks[br].at[b, h, pl.ds(s0 + p * kvr, kvr), :]
            dst = k_buf.at[slot, br, b, pl.ds(p * kvr, kvr), :]
        else:
            src = vs[br].at[b, h, pl.ds(s0 + p * kvr, kvr), :]
            dst = v_buf.at[slot, br, b, pl.ds(p * kvr, kvr), :]
        return pltpu.make_async_copy(src, dst, sems.at[slot, j])

    def start(h, j):
        prio = j % 2
        if isinstance(h, int):
            if h >= nh:
                return
            if h * nsub + j >= total - _TAIL_FIFO:
                prio = 1
        copy(h, j).start(priority=prio)

    def start_global(i):
        if i < nwq:
            wq_copy(i).start(priority=i % 2)
        else:
            start((i - nwq) // nsub, (i - nwq) % nsub)

    x_copies = [pltpu.make_async_copy(xs[br], x_buf.at[br], x_sem.at[br]) for br in range(2)]
    for c in x_copies:
        c.start()
    for i in range(L):
        start_global(i)
    acc[...] = jnp.zeros_like(acc)
    for c in x_copies:
        c.wait()

    for i in range(nwq):
        br, r0, c0, closes = wq_subs[i]
        wq_copy(i).wait()
        start_global(i + L)
        if closes:
            kb = r0 + _WQ_ROWS - _WQ_KB
            part = jnp.dot(x_buf[br, :, kb:kb + _WQ_KB],
                           wq_buf[br, kb:kb + _WQ_KB, c0:c0 + _WQ_COLS],
                           preferred_element_type=jnp.float32)
            if kb == 0:
                q_acc[br, :, c0:c0 + _WQ_COLS] = part
            else:
                q_acc[br, :, c0:c0 + _WQ_COLS] += part

    def step(h, carry):
        slot = h % _NSLOT
        col = h * dh if isinstance(h, int) else pl.multiple_of(h * dh, dh)
        qs = [q_acc[r, :, pl.ds(col, dh)].astype(jnp.bfloat16) for r in range(2)]
        scores, es, ps, outs = {}, {}, {}, {}

        def softmax_num(key):
            s = scores.pop(key)
            e = jnp.exp(s - jnp.max(s, axis=-1, keepdims=True))
            es[key] = e
            ps[key] = e.astype(jnp.bfloat16)

        for j in range(nsub):
            kind, br, b, p, closes = subs[j]
            copy(h, j).wait()
            t = j + L
            start(h + t // nsub, t % nsub)
            if not closes:
                continue
            pending = list(scores)
            if kind == "k":
                scores[br, b] = jax.lax.dot_general(
                    qs[br][b:b + 1, :], k_buf[slot, br, b], (((1,), (1,)), ((), ())),
                    preferred_element_type=jnp.float32) * scale
            elif kind == "v":
                o = jnp.dot(ps[br, b], v_buf[slot, br, b], preferred_element_type=jnp.float32)
                outs[br, b] = o / jnp.sum(es[br, b], axis=-1, keepdims=True)
            else:
                for r in range(2):
                    o_all = jnp.concatenate([outs[r, c] for c in range(nb)], axis=0)
                    acc[r] += jnp.dot(o_all.astype(jnp.bfloat16), wo_buf[slot, r],
                                      preferred_element_type=jnp.float32)
            for key in pending:
                softmax_num(key)
        return carry

    n_peel = -(-(L + _TAIL_FIFO) // nsub)
    jax.lax.fori_loop(0, nh - n_peel, step, 0)
    for h in range(nh - n_peel, nh):
        step(h, 0)
    o_ref[:, 0:d] = acc[0].astype(o_ref.dtype)
    o_ref[:, d:2 * d] = acc[1].astype(o_ref.dtype)


@jax.jit
def pallas_concat_heads__sliding_block_cached__sliding_block_cached__decode_kernel(
    A_x, A_k_cache, A_v_cache, A_wq, A_wo, B_x, B_k_cache, B_v_cache, B_wq, B_wo,
):
    B, Sq, D = A_x.shape
    _, H, Sk, Dh = A_k_cache.shape
    W = min(4096, max(256, Sk // 4))
    assert Sq == 1
    scale = Dh ** -0.5
    nsub = 2 * (_WO_SPLIT + 2 * B * _KV_SPLIT)
    dt = A_x.dtype
    NS = _NSLOT

    any_spec = pl.BlockSpec(memory_space=pl.ANY)

    out = pl.pallas_call(
        functools.partial(_kernel, nb=B, nh=H, dh=Dh, d=D, w=W, s0=Sk - W, scale=scale),
        in_specs=[any_spec] * 10,
        out_specs=pl.BlockSpec((B, 2 * D), lambda: (0, 0)),
        out_shape=jax.ShapeDtypeStruct((B, 2 * D), dt),
        scratch_shapes=[
            pltpu.VMEM((2, B, D), dt),
            pltpu.VMEM((2, D, H * Dh), dt),
            pltpu.VMEM((NS, 2, B, W, Dh), dt),
            pltpu.VMEM((NS, 2, B, W, Dh), dt),
            pltpu.VMEM((NS, 2, Dh, D), dt),
            pltpu.VMEM((2, B, H * Dh), jnp.float32),
            pltpu.VMEM((2, B, D), jnp.float32),
            pltpu.SemaphoreType.DMA((2,)),
            pltpu.SemaphoreType.DMA((_WQ_SEMS,)),
            pltpu.SemaphoreType.DMA((NS, nsub)),
        ],
        compiler_params=pltpu.CompilerParams(vmem_limit_bytes=64 * 1024 * 1024, disable_semaphore_checks=True, disable_bounds_checks=True),
    )(A_x.reshape(B, D), A_k_cache, A_v_cache, A_wq, A_wo, B_x.reshape(B, D), B_k_cache, B_v_cache, B_wq, B_wo)
    return out.reshape(B, Sq, 2 * D)
```

```python
import functools

import jax
import jax.numpy as jnp
import jax.experimental.pallas as pl
import jax.experimental.pallas.tpu as pltpu

_KV_SPLIT = 8
_WO_SPLIT = 4
_LOOKAHEAD = 72
_TAIL_GROUPS = 2
_NSLOT = 2
_WQ_ROWS = 8
_WQ_COLS = 2048
_WQ_KB = 128
_WQ_SEMS = 128


def _kernel(ax, ak, av, awq, awo, bx, bk, bv, bwq, bwo, o_ref,
            x_buf, wq_buf, k_buf, v_buf, wo_buf, q_acc, acc, x_sem, wq_sems, sems,
            *, nb, nh, dh, d, w, s0, scale):
    xs, ks, vs, wqs, wos = (ax, bx), (ak, bk), (av, bv), (awq, bwq), (awo, bwo)
    kvr = w // _KV_SPLIT
    wor = dh // _WO_SPLIT
    L = _LOOKAHEAD
    assert L < _WQ_SEMS and L % 2 == 0

    wq_subs = [(br, kb + rr, cc, rr == _WQ_KB - _WQ_ROWS)
               for br in range(2) for kb in range(0, d, _WQ_KB)
               for cc in range(0, nh * dh, _WQ_COLS) for rr in range(0, _WQ_KB, _WQ_ROWS)]
    nwq = len(wq_subs)
    assert nwq % 2 == 0

    groups = [(kind, b, _KV_SPLIT) for kind in ("k", "v") for b in range(nb)]
    groups.append(("wo", 0, _WO_SPLIT))
    subs = [(kind, br, b, p) for kind, b, n in groups for p in range(n) for br in range(2)]
    nsub = len(subs)
    assert L <= (_NSLOT - 1) * nsub
    group_j0 = [sum(2 * n for _, _, n in groups[:g]) for g in range(len(groups))]
    n_pair_groups = len(groups) - _TAIL_GROUPS
    tail_j0 = group_j0[n_pair_groups] if _TAIL_GROUPS else nsub
    last_order = list(range(tail_j0))
    for g in range(n_pair_groups, len(groups)):
        for br in range(2):
            last_order += [group_j0[g] + 2 * p + br for p in range(groups[g][2])]
    assert L >= nsub - tail_j0

    def wq_copy(i):
        br, r0, c0, _ = wq_subs[i]
        return pltpu.make_async_copy(
            wqs[br].at[pl.ds(r0, _WQ_ROWS), pl.ds(c0, _WQ_COLS)],
            wq_buf.at[br, pl.ds(r0, _WQ_ROWS), pl.ds(c0, _WQ_COLS)],
            wq_sems.at[i % _WQ_SEMS])

    def copy(h, j):
        kind, br, b, p = subs[j]
        slot = h % _NSLOT
        if kind == "wo":
            src = wos[br].at[pl.ds(pl.multiple_of(h * dh + p * wor, wor), wor), :]
            dst = wo_buf.at[slot, br, pl.ds(p * wor, wor), :]
        elif kind == "k":
            src = ks[br].at[b, h, pl.ds(s0 + p * kvr, kvr), :]
            dst = k_buf.at[slot, br, b, pl.ds(p * kvr, kvr), :]
        else:
            src = vs[br].at[b, h, pl.ds(s0 + p * kvr, kvr), :]
            dst = v_buf.at[slot, br, b, pl.ds(p * kvr, kvr), :]
        return pltpu.make_async_copy(src, dst, sems.at[slot, j])

    def start(h, pos):
        j, prio = pos, pos % 2
        if isinstance(h, int):
            if h >= nh:
                return
            if h == nh - 1 and pos >= tail_j0:
                j, prio = last_order[pos], 1
        copy(h, j).start(priority=prio)

    def start_global(i):
        if i < nwq:
            wq_copy(i).start(priority=i % 2)
        else:
            start((i - nwq) // nsub, (i - nwq) % nsub)

    x_copies = [pltpu.make_async_copy(xs[br], x_buf.at[br], x_sem.at[br]) for br in range(2)]
    for c in x_copies:
        c.start()
    for i in range(L):
        start_global(i)
    acc[...] = jnp.zeros_like(acc)

    for i in range(nwq):
        br, r0, c0, closes = wq_subs[i]
        wq_copy(i).wait()
        start_global(i + L)
        if closes:
            kb = r0 + _WQ_ROWS - _WQ_KB
            if kb == 0 and c0 == 0:
                x_copies[br].wait()
            part = jnp.dot(x_buf[br, :, kb:kb + _WQ_KB],
                           wq_buf[br, kb:kb + _WQ_KB, c0:c0 + _WQ_COLS],
                           preferred_element_type=jnp.float32)
            if kb == 0:
                q_acc[br, :, c0:c0 + _WQ_COLS] = part
            else:
                q_acc[br, :, c0:c0 + _WQ_COLS] += part

    def step(h, carry):
        static = isinstance(h, int)
        slot = h % _NSLOT
        is_last = static and h == nh - 1
        col = h * dh if static else pl.multiple_of(h * dh, dh)
        qs = [q_acc[r, :, pl.ds(col, dh)].astype(jnp.bfloat16) for r in range(2)]
        scores, es, ps, outs = {}, {}, {}, {}

        def compute(kind, br, b):
            pending = list(scores)
            if kind == "k":
                scores[br, b] = jax.lax.dot_general(
                    qs[br][b:b + 1, :], k_buf[slot, br, b], (((1,), (1,)), ((), ())),
                    preferred_element_type=jnp.float32) * scale
            elif kind == "v":
                o = jnp.dot(ps[br, b], v_buf[slot, br, b], preferred_element_type=jnp.float32)
                outs[br, b] = o / jnp.sum(es[br, b], axis=-1, keepdims=True)
            else:
                o_all = jnp.concatenate([outs[br, c] for c in range(nb)], axis=0)
                res = acc[br] + jnp.dot(o_all.astype(jnp.bfloat16), wo_buf[slot, br],
                                        preferred_element_type=jnp.float32)
                if is_last:
                    o_ref[:, br * d:(br + 1) * d] = res.astype(o_ref.dtype)
                else:
                    acc[br] = res
            for key in pending:
                s = scores.pop(key)
                e = jnp.exp(s - jnp.max(s, axis=-1, keepdims=True))
                es[key] = e
                ps[key] = e.astype(jnp.bfloat16)

        for g, (kind, b, n) in enumerate(groups):
            j0 = group_j0[g]
            if is_last and g >= n_pair_groups:
                for br in range(2):
                    for p in range(n):
                        copy(h, j0 + 2 * p + br).wait()
                    compute(kind, br, b)
                continue
            for p in range(n):
                copy(h, j0 + 2 * p).wait()
            for p in range(n):
                copy(h, j0 + 2 * p + 1).wait()
                ta, tb = j0 + 2 * p + L, j0 + 2 * p + 1 + L
                for t in ((ta, tb) if static else (tb, ta)):
                    start(h + t // nsub, t % nsub)
                if p == n // 2 - 1:
                    compute(kind, 0, b)
            compute(kind, 1, b)
        return carry

    n_peel = -(-L // nsub) + 1
    jax.lax.fori_loop(0, nh - n_peel, step, 0)
    for h in range(nh - n_peel, nh):
        step(h, 0)


@jax.jit
def pallas_concat_heads__sliding_block_cached__sliding_block_cached__decode_kernel(
    A_x: jax.Array,
    A_k_cache: jax.Array,
    A_v_cache: jax.Array,
    A_wq: jax.Array,
    A_wo: jax.Array,
    B_x: jax.Array,
    B_k_cache: jax.Array,
    B_v_cache: jax.Array,
    B_wq: jax.Array,
    B_wo: jax.Array,
):
    B, Sq, D = A_x.shape
    _, H, Sk, Dh = A_k_cache.shape
    W = min(4096, max(256, Sk // 4))
    assert Sq == 1 and A_wq.shape == (D, H * Dh) and A_wo.shape == (H * Dh, D)
    assert W % _KV_SPLIT == 0 and Dh % _WO_SPLIT == 0
    assert D % _WQ_KB == 0 and (H * Dh) % _WQ_COLS == 0
    scale = Dh ** -0.5
    nsub = 2 * (_WO_SPLIT + 2 * B * _KV_SPLIT)
    dt = A_x.dtype

    out = pl.pallas_call(
        functools.partial(_kernel, nb=B, nh=H, dh=Dh, d=D, w=W, s0=Sk - W, scale=scale),
        in_specs=[pl.BlockSpec(memory_space=pl.ANY)] * 10,
        out_specs=pl.BlockSpec((B, 2 * D), lambda: (0, 0)),
        out_shape=jax.ShapeDtypeStruct((B, 2 * D), dt),
        scratch_shapes=[
            pltpu.VMEM((2, B, D), dt),
            pltpu.VMEM((2, D, H * Dh), dt),
            pltpu.VMEM((_NSLOT, 2, B, W, Dh), dt),
            pltpu.VMEM((_NSLOT, 2, B, W, Dh), dt),
            pltpu.VMEM((_NSLOT, 2, Dh, D), dt),
            pltpu.VMEM((2, B, H * Dh), jnp.float32),
            pltpu.VMEM((2, B, D), jnp.float32),
            pltpu.SemaphoreType.DMA((2,)),
            pltpu.SemaphoreType.DMA((_WQ_SEMS,)),
            pltpu.SemaphoreType.DMA((_NSLOT, nsub)),
        ],
        compiler_params=pltpu.CompilerParams(
            vmem_limit_bytes=64 * 1024 * 1024,
            disable_semaphore_checks=True,
            disable_bounds_checks=True,
        ),
    )(A_x.reshape(B, D), A_k_cache, A_v_cache, A_wq, A_wo,
      B_x.reshape(B, D), B_k_cache, B_v_cache, B_wq, B_wo)
    return out.reshape(B, Sq, 2 * D)
```
